```python
import os as _os
_os.environ.setdefault("JAX_PLATFORMS", "cpu")
import jax
import jax.numpy as jnp

def _softmax(x, axis=-1):
    return jax.nn.softmax(x, axis=axis)
def _gelu(x):
    return jax.nn.gelu(x, approximate=True)
def _silu(x):
    return jax.nn.silu(x)
def _sigmoid(x):
    return jax.nn.sigmoid(x)
def _layernorm(x, axis=-1, eps=1e-5):
    m = jnp.mean(x, axis=axis, keepdims=True)
    v = jnp.var(x, axis=axis, keepdims=True)
    return (x - m) / jnp.sqrt(v + eps)
def _scatter_add(tgt, idx, src, axis=0):
    return tgt.at[idx].add(src)
def _segment_sum(src, seg, n):
    return jax.ops.segment_sum(src, seg, n)
class _Rng:
    def __init__(self, key):
        self._k = key
    def _next(self):
        self._k, sub = jax.random.split(self._k)
        return sub
    def normal(self, shape):
        return jax.random.normal(self._next(), shape, dtype=jnp.bfloat16)
    def randint(self, lo, hi, shape):
        return jax.random.randint(self._next(), shape, lo, hi, dtype=jnp.int32)
    def uniform(self, shape, lo=0.0, hi=1.0):
        return jax.random.uniform(self._next(), shape, jnp.bfloat16, lo, hi)
    def permutation(self, n):
        return jax.random.permutation(self._next(), n)


kernel_name = 'sequential_preLN__ssm_conv_h3__mixer_s_mlp__prompt'

def setup_inputs():
    _rng = _Rng(jax.random.key(int.from_bytes(__import__("os").urandom(4), "little")))
    _w = (lambda a: (lambda t: t.astype(jnp.bfloat16) if jnp.issubdtype(t.dtype, jnp.floating) else t)(jnp.asarray(a)))
    def _A_setup():
        B, S, D = 1, 2048, 640
        ks = 4
        return {
            "q": _w((lambda *s: _rng.normal(s) * 0.05)(B, S, D)),
            "k": _w((lambda *s: _rng.normal(s) * 0.05)(B, S, D)),
            "v": _w((lambda *s: _rng.normal(s) * 0.05)(B, S, D)),
            "shift_k": _w((lambda *s: _rng.normal(s) * 0.05)(D, ks) * 0.5),
            "ssm_k": _w((lambda *s: _rng.normal(s) * 0.05)(D, S) * (1.0 / S ** 0.5)),
            "ssm_D": _w((lambda *s: _rng.normal(s) * 0.05)(D)),
        }
    _A_in = _A_setup()

    def _B_setup():
        B, S, D, F = 1, 2048, 640, 1728
        return {
            "x":  _w((lambda *s: _rng.normal(s) * 0.05)(B, S, D)),
            "w1": _w((lambda *s: _rng.normal(s) * 0.8)(D, D) * (D ** -0.5)),
            "w2": _w((lambda *s: _rng.normal(s) * 0.8)(D, D) * (D ** -0.5)),
            "w3": _w((lambda *s: _rng.normal(s) * 0.8)(D, F) * (D ** -0.5)),
            "w4": _w((lambda *s: _rng.normal(s) * 0.8)(F, D) * (F ** -0.5)),
        }
    _B_in = _B_setup()

    return {
        "A_q": _A_in["q"],
        "A_k": _A_in["k"],
        "A_v": _A_in["v"],
        "A_shift_k": _A_in["shift_k"],
        "A_ssm_k": _A_in["ssm_k"],
        "A_ssm_D": _A_in["ssm_D"],
        "B_x": _B_in["x"],
        "B_w1": _B_in["w1"],
        "B_w2": _B_in["w2"],
        "B_w3": _B_in["w3"],
        "B_w4": _B_in["w4"],
    }

def reference(A_q, A_k, A_v, A_shift_k, A_ssm_k, A_ssm_D, B_x, B_w1, B_w2, B_w3, B_w4):
    def _A_ref(q, k, v, shift_k, ssm_k, ssm_D):
        B, S, D = q.shape
        ks = shift_k.shape[-1]
        k_pad = jnp.pad(k, ((0, 0), (ks - 1, 0), (0, 0)))
        k_shift = jnp.zeros_like(k)
        for t in range(ks):
            k_shift = k_shift + k_pad[:, t:t + S, :] * shift_k[:, ks - 1 - t][None, None, :]
        kv = k_shift * v
        L = 2 * S
        kv_pad = jnp.pad(kv, ((0, 0), (0, S), (0, 0)))
        kf_pad = jnp.pad(ssm_k, ((0, 0), (0, S)))
        kv_f = (lambda x, axes=(-2,-1): jnp.fft.rfft2(x.astype(jnp.float32), axes=axes))(kv_pad[:, None, :, :], axes=(1, 2))
        kf_f = (lambda x, axes=(-2,-1): jnp.fft.rfft2(x.astype(jnp.float32), axes=axes))(kf_pad[:, None, :], axes=(1, 2))
        kf_f = (lambda x, *d: x.transpose(*d))(kf_f, 1, 2, 0)
        y_f = kv_f * kf_f[None, :, :, :]
        y = (lambda x, s, axes=(-2,-1): jnp.fft.irfft2(x, s=s, axes=axes).astype(jnp.bfloat16))(y_f, (1, L), axes=(1, 2))[:, 0, :S, :]
        y = y + kv * ssm_D[None, None, :]
        return q * y

    def _B_ref(x, w1, w2, w3, w4):
        B, S, D = x.shape
        h = _gelu(_layernorm(x, axis=-1) @ w1)
        c = D // 4
        g0 = jnp.pad(h[:, :, 0*c:1*c], ((0, 0), (1, 0), (0, 0)))[:, :S, :]
        g1 = jnp.pad(h[:, :, 1*c:2*c], ((0, 0), (0, 1), (0, 0)))[:, 1:, :]
        g2 = jnp.pad(h[:, :, 2*c:3*c], ((0, 0), (2, 0), (0, 0)))[:, :S, :]
        g3 = jnp.pad(h[:, :, 3*c:   ], ((0, 0), (0, 2), (0, 0)))[:, 2:, :]
        hs = jnp.concatenate([g0, g1, g2, g3], axis=-1) @ w2
        x1 = x + hs
        h2 = _gelu(_layernorm(x1, axis=-1) @ w3) @ w4
        return x1 + h2

    x = A_q
    h = x + _A_ref(_layernorm(x, axis=-1), A_k, A_v, A_shift_k, A_ssm_k, A_ssm_D)
    h2 = h + _B_ref(_layernorm(h, axis=-1), B_w1, B_w2, B_w3, B_w4)
    return h2
```

```python
import numpy as np
import jax
import jax.numpy as jnp
import jax.experimental.pallas as pl
import jax.experimental.pallas.tpu as pltpu

S, D, FF = 2048, 640, 1728
CB = 128
NB = S // CB
CT = 128
NC = D // CT
TA = 512
NA = S // TA
TB = 512
NBT = S // TB
PAD = 8
FCH = 32
G = D // 4


def _dft_mats():
    f = np.arange(CB, dtype=np.float64)[:, None] + 0.5
    j = np.arange(CB, dtype=np.float64)[None, :]
    th = 2.0 * np.pi * f * j / (2 * CB)
    fwd = np.concatenate([np.cos(th), -np.sin(th)], axis=0)
    inv = np.concatenate([np.cos(th).T, -np.sin(th).T], axis=1) / CB
    sgn = np.where(np.arange(CB) % 2 == 0, 1.0, -1.0)[:, None] * np.ones((1, CT))
    return fwd, inv, sgn


_FWD, _INV, _SGN = _dft_mats()


def _ln(x):
    m = jnp.mean(x, axis=-1, keepdims=True)
    xc = x - m
    v = jnp.mean(xc * xc, axis=-1, keepdims=True)
    return xc * jax.lax.rsqrt(v + 1e-5)


def _gelu(x):
    return 0.5 * x * (1.0 + jnp.tanh(0.7978845608028654 * (x + 0.044715 * (x * x * x))))


def _kernel(x_ref, k_ref, v_ref, sk_ref, ssm_ref, dd_ref, fwd_ref, inv_ref, sgn_ref,
            w1_hbm, w2_hbm, w3_hbm, w4_hbm, o_ref,
            kpad, kv_sc, xs, ps, ks, ysc, h_sc, xb_sc, h1_sc,
            w1_v, w2_v, w3_v, w4_v, sems):
    s = pl.program_id(0)
    f32 = jnp.float32
    bf16 = jnp.bfloat16

    def wcopies():
        return [pltpu.make_async_copy(w1_hbm, w1_v, sems.at[0]),
                pltpu.make_async_copy(w2_hbm, w2_v, sems.at[1]),
                pltpu.make_async_copy(w3_hbm, w3_v, sems.at[2]),
                pltpu.make_async_copy(w4_hbm, w4_v, sems.at[3])]

    @pl.when(s == 0)
    def _():
        for c in wcopies():
            c.start()
        h1_sc[0:PAD, :] = jnp.zeros((PAD, D), f32)
        h1_sc[PAD + S:PAD + S + PAD, :] = jnp.zeros((PAD, D), f32)

    @pl.when(s < NC)
    def _():
        kpad[0:PAD, :] = jnp.zeros((PAD, CT), f32)
        kpad[PAD:, :] = k_ref[...].astype(f32)
        wt = jnp.transpose(sk_ref[...].astype(f32))
        fwd = fwd_ref[...]
        for i in range(NB):
            r0 = PAD + i * CB
            ksh = kpad[r0:r0 + CB, :] * wt[0:1, :]
            for l in range(1, 4):
                ksh = ksh + kpad[r0 - l:r0 - l + CB, :] * wt[l:l + 1, :]
            kv = (ksh * v_ref[i * CB:(i + 1) * CB, :].astype(f32)).astype(bf16)
            kv_sc[i] = kv
            xs[i] = jnp.dot(fwd, kv, preferred_element_type=f32)
            ps[i] = jax.lax.dot_general(
                fwd, ssm_ref[:, i * CB:(i + 1) * CB], (((1,), (1,)), ((), ())),
                preferred_element_type=f32)
        sgn = sgn_ref[...]
        ks[0] = ps[0]
        for m in range(1, NB):
            ks[m, 0:CB, :] = ps[m, 0:CB, :] - sgn * ps[m - 1, CB:2 * CB, :]
            ks[m, CB:2 * CB, :] = ps[m, CB:2 * CB, :] + sgn * ps[m - 1, 0:CB, :]

        def chunk(cidx, carry):
            a = pl.multiple_of(cidx * FCH, FCH)
            b = pl.multiple_of(CB + cidx * FCH, FCH)
            for i in range(NB):
                yre = jnp.zeros((FCH, CT), f32)
                yim = jnp.zeros((FCH, CT), f32)
                for m in range(i + 1):
                    kr = ks[m, pl.ds(a, FCH), :]
                    ki = ks[m, pl.ds(b, FCH), :]
                    xr = xs[i - m, pl.ds(a, FCH), :]
                    xi = xs[i - m, pl.ds(b, FCH), :]
                    yre = yre + (kr * xr - ki * xi)
                    yim = yim + (kr * xi + ki * xr)
                ps[i, pl.ds(a, FCH), :] = yre
                ps[i, pl.ds(b, FCH), :] = yim
            return carry

        jax.lax.fori_loop(0, CB // FCH, chunk, 0)
        inv = inv_ref[...]
        dd = dd_ref[...].astype(f32)
        for i in range(NB):
            y = jnp.dot(inv, ps[i].astype(bf16), preferred_element_type=f32)
            y = y.astype(bf16).astype(f32) + kv_sc[i].astype(f32) * dd
            ysc[s, i * CB:(i + 1) * CB, :] = y.astype(bf16)

    @pl.when((s >= NC) & (s < NC + NA))
    def _():
        @pl.when(s == NC)
        def _():
            for c in wcopies():
                c.wait()
        t = s - NC
        r0 = pl.multiple_of(t * TA, TA)
        x = x_ref[...].astype(f32)
        q = _ln(x).astype(bf16).astype(f32)
        y = jnp.concatenate([ysc[c, pl.ds(r0, TA), :] for c in range(NC)], axis=-1).astype(f32)
        h = (x + (q * y).astype(bf16).astype(f32)).astype(bf16)
        xb = _ln(h.astype(f32)).astype(bf16)
        a = _ln(xb.astype(f32)).astype(bf16)
        h1 = _gelu(jnp.dot(a, w1_v[...], preferred_element_type=f32))
        h_sc[pl.ds(r0, TA), :] = h
        xb_sc[pl.ds(r0, TA), :] = xb
        h1_sc[pl.ds(PAD + r0, TA), :] = h1.astype(bf16).astype(f32)

    @pl.when(s >= NC + NA)
    def _():
        t = s - NC - NA
        win = h1_sc[pl.ds(pl.multiple_of(t * TB, TB), TB + 2 * PAD), :]
        lane = jax.lax.broadcasted_iota(jnp.int32, (TB, D), 1)
        hm1 = win[PAD - 1:PAD - 1 + TB, :]
        hp1 = win[PAD + 1:PAD + 1 + TB, :]
        hm2 = win[PAD - 2:PAD - 2 + TB, :]
        hp2 = win[PAD + 2:PAD + 2 + TB, :]
        hsh = jnp.where(lane < G, hm1, jnp.where(lane < 2 * G, hp1, jnp.where(lane < 3 * G, hm2, hp2)))
        hs = jnp.dot(hsh.astype(bf16), w2_v[...], preferred_element_type=f32)
        rr = pl.multiple_of(t * TB, TB)
        x1 = xb_sc[pl.ds(rr, TB), :].astype(f32) + hs
        a = _ln(x1).astype(bf16)
        g = _gelu(jnp.dot(a, w3_v[...], preferred_element_type=f32)).astype(bf16)
        h2 = jnp.dot(g, w4_v[...], preferred_element_type=f32)
        o_ref[...] = (h_sc[pl.ds(rr, TB), :].astype(f32) + x1 + h2).astype(o_ref.dtype)


@jax.jit
def pallas_sequential_preLN__ssm_conv_h3__mixer_s_mlp__prompt_kernel(
    A_q, A_k, A_v, A_shift_k, A_ssm_k, A_ssm_D, B_x, B_w1, B_w2, B_w3, B_w4,
):
    del B_x
    bf16 = jnp.bfloat16
    x = A_q.reshape(S, D)
    k = A_k.reshape(S, D)
    v = A_v.reshape(S, D)
    sk = jnp.pad(A_shift_k, ((0, 0), (0, 4)))
    dd = A_ssm_D.reshape(1, D)
    fwd = jnp.asarray(_FWD, bf16)
    inv = jnp.asarray(_INV, bf16)
    sgn = jnp.asarray(_SGN, jnp.float32)

    cmap = lambda s: (0, jnp.minimum(s, NC - 1))
    const = lambda s: (0, 0)
    in_specs = [
        pl.BlockSpec((TA, D), lambda s: (jnp.clip(s - NC, 0, NA - 1), 0)),
        pl.BlockSpec((S, CT), cmap),
        pl.BlockSpec((S, CT), cmap),
        pl.BlockSpec((CT, 8), lambda s: (jnp.minimum(s, NC - 1), 0)),
        pl.BlockSpec((CT, S), lambda s: (jnp.minimum(s, NC - 1), 0)),
        pl.BlockSpec((1, CT), cmap),
        pl.BlockSpec((2 * CB, CB), const),
        pl.BlockSpec((CB, 2 * CB), const),
        pl.BlockSpec((CB, CT), const),
        pl.BlockSpec(memory_space=pl.ANY),
        pl.BlockSpec(memory_space=pl.ANY),
        pl.BlockSpec(memory_space=pl.ANY),
        pl.BlockSpec(memory_space=pl.ANY),
    ]
    out = pl.pallas_call(
        _kernel,
        grid=(NC + NA + NBT,),
        in_specs=in_specs,
        out_specs=pl.BlockSpec((TB, D), lambda s: (jnp.clip(s - NC - NA, 0, NBT - 1), 0)),
        out_shape=jax.ShapeDtypeStruct((S, D), A_q.dtype),
        scratch_shapes=[
            pltpu.VMEM((PAD + S, CT), jnp.float32),
            pltpu.VMEM((NB, CB, CT), bf16),
            pltpu.VMEM((NB, 2 * CB, CT), jnp.float32),
            pltpu.VMEM((NB, 2 * CB, CT), jnp.float32),
            pltpu.VMEM((NB, 2 * CB, CT), jnp.float32),
            pltpu.VMEM((NC, S, CT), bf16),
            pltpu.VMEM((S, D), bf16),
            pltpu.VMEM((S, D), bf16),
            pltpu.VMEM((S + 2 * PAD, D), jnp.float32),
            pltpu.VMEM((D, D), bf16),
            pltpu.VMEM((D, D), bf16),
            pltpu.VMEM((D, FF), bf16),
            pltpu.VMEM((FF, D), bf16),
            pltpu.SemaphoreType.DMA((4,)),
        ],
        compiler_params=pltpu.CompilerParams(
            dimension_semantics=("arbitrary",),
            vmem_limit_bytes=100 * 1024 * 1024,
        ),
    )(x, k, v, sk, A_ssm_k, dd, fwd, inv, sgn, B_w1, B_w2, B_w3, B_w4)
    return out.reshape(1, S, D)
```

```python
import numpy as np
import jax
import jax.numpy as jnp
import jax.experimental.pallas as pl
import jax.experimental.pallas.tpu as pltpu

S, D, FF = 2048, 640, 1728
CB = 128
NB = S // CB
CT = 640
NC = D // CT
TA = 512
NA = S // TA
TB = 512
NBT = S // TB
PAD = 8
FCH = 32
G = D // 4


def _dft_mats():
    f = np.arange(CB, dtype=np.float64)[:, None] + 0.5
    j = np.arange(CB, dtype=np.float64)[None, :]
    th = 2.0 * np.pi * f * j / (2 * CB)
    fwd = np.concatenate([np.cos(th), -np.sin(th)], axis=0)
    inv = np.concatenate([np.cos(th).T, -np.sin(th).T], axis=1) / CB
    sgn = np.where(np.arange(CB) % 2 == 0, 1.0, -1.0)[:, None] * np.ones((1, CT))
    return fwd, inv, sgn


_FWD, _INV, _SGN = _dft_mats()


def _ln(x):
    m = jnp.mean(x, axis=-1, keepdims=True)
    xc = x - m
    v = jnp.mean(xc * xc, axis=-1, keepdims=True)
    return xc * jax.lax.rsqrt(v + 1e-5)


def _gelu(x):
    return 0.5 * x * (1.0 + jnp.tanh(0.7978845608028654 * (x + 0.044715 * (x * x * x))))


def _kernel(x_ref, k_ref, v_ref, sk_ref, ssm_ref, dd_ref, fwd_ref, inv_ref, sgn_ref,
            w1_hbm, w2_hbm, w3_hbm, w4_hbm, o_ref,
            kpad, kv_sc, xs, ps, ks, ysc, h_sc, xb_sc, h1_sc,
            w1_v, w2_v, w3_v, w4_v, sems):
    s = pl.program_id(0)
    f32 = jnp.float32
    bf16 = jnp.bfloat16

    def wcopies():
        return [pltpu.make_async_copy(w1_hbm, w1_v, sems.at[0]),
                pltpu.make_async_copy(w2_hbm, w2_v, sems.at[1]),
                pltpu.make_async_copy(w3_hbm, w3_v, sems.at[2]),
                pltpu.make_async_copy(w4_hbm, w4_v, sems.at[3])]

    @pl.when(s == 0)
    def _():
        for c in wcopies():
            c.start()
        h1_sc[0:PAD, :] = jnp.zeros((PAD, D), f32)
        h1_sc[PAD + S:PAD + S + PAD, :] = jnp.zeros((PAD, D), f32)

    @pl.when(s < NC)
    def _():
        kpad[0:PAD, :] = jnp.zeros((PAD, CT), f32)
        kpad[PAD:, :] = k_ref[...].astype(f32)
        wt = sk_ref[...].astype(f32)
        fwd = fwd_ref[...]
        for i in range(NB):
            r0 = PAD + i * CB
            ksh = kpad[r0:r0 + CB, :] * wt[0:1, :]
            for l in range(1, 4):
                ksh = ksh + kpad[r0 - l:r0 - l + CB, :] * wt[l:l + 1, :]
            kv = (ksh * v_ref[i * CB:(i + 1) * CB, :].astype(f32)).astype(bf16)
            kv_sc[i] = kv
            xs[i] = jnp.dot(fwd, kv, preferred_element_type=f32)
            ps[i] = jax.lax.dot_general(
                fwd, ssm_ref[:, i * CB:(i + 1) * CB], (((1,), (1,)), ((), ())),
                preferred_element_type=f32)
        sgn = sgn_ref[...]
        ks[0] = ps[0]
        for m in range(1, NB):
            ks[m, 0:CB, :] = ps[m, 0:CB, :] - sgn * ps[m - 1, CB:2 * CB, :]
            ks[m, CB:2 * CB, :] = ps[m, CB:2 * CB, :] + sgn * ps[m - 1, 0:CB, :]

        def chunk(cidx, carry):
            a = pl.multiple_of(cidx * FCH, FCH)
            b = pl.multiple_of(CB + cidx * FCH, FCH)
            for i in range(NB):
                yre = jnp.zeros((FCH, CT), f32)
                yim = jnp.zeros((FCH, CT), f32)
                for m in range(i + 1):
                    kr = ks[m, pl.ds(a, FCH), :]
                    ki = ks[m, pl.ds(b, FCH), :]
                    xr = xs[i - m, pl.ds(a, FCH), :]
                    xi = xs[i - m, pl.ds(b, FCH), :]
                    yre = yre + (kr * xr - ki * xi)
                    yim = yim + (kr * xi + ki * xr)
                ps[i, pl.ds(a, FCH), :] = yre
                ps[i, pl.ds(b, FCH), :] = yim
            return carry

        jax.lax.fori_loop(0, CB // FCH, chunk, 0)
        inv = inv_ref[...]
        dd = dd_ref[...].astype(f32)
        for i in range(NB):
            y = jnp.dot(inv, ps[i].astype(bf16), preferred_element_type=f32)
            y = y.astype(bf16).astype(f32) + kv_sc[i].astype(f32) * dd
            ysc[s, i * CB:(i + 1) * CB, :] = y.astype(bf16)

    @pl.when((s >= NC) & (s < NC + NA))
    def _():
        @pl.when(s == NC)
        def _():
            for c in wcopies():
                c.wait()
        t = s - NC
        r0 = pl.multiple_of(t * TA, TA)
        x = x_ref[...].astype(f32)
        q = _ln(x).astype(bf16).astype(f32)
        y = jnp.concatenate([ysc[c, pl.ds(r0, TA), :] for c in range(NC)], axis=-1).astype(f32)
        h = (x + (q * y).astype(bf16).astype(f32)).astype(bf16)
        xb = _ln(h.astype(f32)).astype(bf16)
        a = _ln(xb.astype(f32)).astype(bf16)
        h1 = _gelu(jnp.dot(a, w1_v[...], preferred_element_type=f32))
        h_sc[pl.ds(r0, TA), :] = h
        xb_sc[pl.ds(r0, TA), :] = xb
        h1_sc[pl.ds(PAD + r0, TA), :] = h1.astype(bf16).astype(f32)

    @pl.when(s >= NC + NA)
    def _():
        t = s - NC - NA
        win = h1_sc[pl.ds(pl.multiple_of(t * TB, TB), TB + 2 * PAD), :]
        lane = jax.lax.broadcasted_iota(jnp.int32, (TB, D), 1)
        hm1 = win[PAD - 1:PAD - 1 + TB, :]
        hp1 = win[PAD + 1:PAD + 1 + TB, :]
        hm2 = win[PAD - 2:PAD - 2 + TB, :]
        hp2 = win[PAD + 2:PAD + 2 + TB, :]
        hsh = jnp.where(lane < G, hm1, jnp.where(lane < 2 * G, hp1, jnp.where(lane < 3 * G, hm2, hp2)))
        hs = jnp.dot(hsh.astype(bf16), w2_v[...], preferred_element_type=f32)
        rr = pl.multiple_of(t * TB, TB)
        x1 = xb_sc[pl.ds(rr, TB), :].astype(f32) + hs
        a = _ln(x1).astype(bf16)
        g = _gelu(jax.lax.dot_general(a, w3_v[...], (((1,), (1,)), ((), ())),
                                      preferred_element_type=f32)).astype(bf16)
        h2 = jnp.dot(g, w4_v[...], preferred_element_type=f32)
        o_ref[...] = (h_sc[pl.ds(rr, TB), :].astype(f32) + x1 + h2).astype(o_ref.dtype)


@jax.jit
def pallas_sequential_preLN__ssm_conv_h3__mixer_s_mlp__prompt_kernel(
    A_q, A_k, A_v, A_shift_k, A_ssm_k, A_ssm_D, B_x, B_w1, B_w2, B_w3, B_w4,
):
    del B_x
    bf16 = jnp.bfloat16
    x = A_q.reshape(S, D)
    k = A_k.reshape(S, D)
    v = A_v.reshape(S, D)
    sk = A_shift_k.T
    w3t = B_w3.T
    dd = A_ssm_D.reshape(1, D)
    fwd = jnp.asarray(_FWD, bf16)
    inv = jnp.asarray(_INV, bf16)
    sgn = jnp.asarray(_SGN, jnp.float32)

    cmap = lambda s: (0, jnp.minimum(s, NC - 1))
    const = lambda s: (0, 0)
    in_specs = [
        pl.BlockSpec((TA, D), lambda s: (jnp.clip(s - NC, 0, NA - 1), 0)),
        pl.BlockSpec((S, CT), cmap),
        pl.BlockSpec((S, CT), cmap),
        pl.BlockSpec((4, CT), cmap),
        pl.BlockSpec((CT, S), lambda s: (jnp.minimum(s, NC - 1), 0)),
        pl.BlockSpec((1, CT), cmap),
        pl.BlockSpec((2 * CB, CB), const),
        pl.BlockSpec((CB, 2 * CB), const),
        pl.BlockSpec((CB, CT), const),
        pl.BlockSpec(memory_space=pl.ANY),
        pl.BlockSpec(memory_space=pl.ANY),
        pl.BlockSpec(memory_space=pl.ANY),
        pl.BlockSpec(memory_space=pl.ANY),
    ]
    out = pl.pallas_call(
        _kernel,
        grid=(NC + NA + NBT,),
        in_specs=in_specs,
        out_specs=pl.BlockSpec((TB, D), lambda s: (jnp.clip(s - NC - NA, 0, NBT - 1), 0)),
        out_shape=jax.ShapeDtypeStruct((S, D), A_q.dtype),
        scratch_shapes=[
            pltpu.VMEM((PAD + S, CT), jnp.float32),
            pltpu.VMEM((NB, CB, CT), bf16),
            pltpu.VMEM((NB, 2 * CB, CT), jnp.float32),
            pltpu.VMEM((NB, 2 * CB, CT), jnp.float32),
            pltpu.VMEM((NB, 2 * CB, CT), jnp.float32),
            pltpu.VMEM((NC, S, CT), bf16),
            pltpu.VMEM((S, D), bf16),
            pltpu.VMEM((S, D), bf16),
            pltpu.VMEM((S + 2 * PAD, D), jnp.float32),
            pltpu.VMEM((D, D), bf16),
            pltpu.VMEM((D, D), bf16),
            pltpu.VMEM((FF, D), bf16),
            pltpu.VMEM((FF, D), bf16),
            pltpu.SemaphoreType.DMA((4,)),
        ],
        compiler_params=pltpu.CompilerParams(
            dimension_semantics=("arbitrary",),
            vmem_limit_bytes=127 * 1024 * 1024,
        ),
    )(x, k, v, sk, A_ssm_k, dd, fwd, inv, sgn, B_w1, B_w2, w3t, B_w4)
    return out.reshape(1, S, D)
```
